```python
import os as _os
_os.environ.setdefault("JAX_PLATFORMS", "cpu")
import jax
import jax.numpy as jnp

def _softmax(x, axis=-1):
    return jax.nn.softmax(x, axis=axis)
def _gelu(x):
    return jax.nn.gelu(x, approximate=True)
def _silu(x):
    return jax.nn.silu(x)
def _sigmoid(x):
    return jax.nn.sigmoid(x)
def _layernorm(x, axis=-1, eps=1e-5):
    m = jnp.mean(x, axis=axis, keepdims=True)
    v = jnp.var(x, axis=axis, keepdims=True)
    return (x - m) / jnp.sqrt(v + eps)
def _scatter_add(tgt, idx, src, axis=0):
    return tgt.at[idx].add(src)
def _segment_sum(src, seg, n):
    return jax.ops.segment_sum(src, seg, n)
class _Rng:
    def __init__(self, key):
        self._k = key
    def _next(self):
        self._k, sub = jax.random.split(self._k)
        return sub
    def normal(self, shape):
        return jax.random.normal(self._next(), shape, dtype=jnp.bfloat16)
    def randint(self, lo, hi, shape):
        return jax.random.randint(self._next(), shape, lo, hi, dtype=jnp.int32)
    def uniform(self, shape, lo=0.0, hi=1.0):
        return jax.random.uniform(self._next(), shape, jnp.bfloat16, lo, hi)
    def permutation(self, n):
        return jax.random.permutation(self._next(), n)


kernel_name = 'sequential_preLN__mha_block__swiglu_ffn__prompt'

def setup_inputs():
    _rng = _Rng(jax.random.key(int.from_bytes(__import__("os").urandom(4), "little")))
    _w = (lambda a: (lambda t: t.astype(jnp.bfloat16) if jnp.issubdtype(t.dtype, jnp.floating) else t)(jnp.asarray(a)))
    def _A_setup():
        B, S, D, H = 1, 2048, 640, 32
        return {
            "x": _w((lambda *s: _rng.normal(s) * 0.05)(B, S, D)),
            "wqkv": _w((lambda *s: _rng.normal(s) * 0.05)(D, 3 * D)),
            "wo": _w((lambda *s: _rng.normal(s) * 0.05)(D, D)),
        }
    _A_in = _A_setup()

    def _B_setup():
        B, S, D, F = 1, 2048, 640, 1728
        return {
            "x": _w((lambda *s: _rng.normal(s) * 0.05)(B, S, D)),
            "w_gate": _w((lambda *s: _rng.normal(s) * 0.05)(D, F)),
            "w_up": _w((lambda *s: _rng.normal(s) * 0.05)(D, F)),
            "w_down": _w((lambda *s: _rng.normal(s) * 0.05)(F, D)),
        }
    _B_in = _B_setup()

    return {
        "A_x": _A_in["x"],
        "A_wqkv": _A_in["wqkv"],
        "A_wo": _A_in["wo"],
        "B_x": _B_in["x"],
        "B_w_gate": _B_in["w_gate"],
        "B_w_up": _B_in["w_up"],
        "B_w_down": _B_in["w_down"],
    }

def reference(A_x, A_wqkv, A_wo, B_x, B_w_gate, B_w_up, B_w_down):
    def _A_ref(x, wqkv, wo):
        B, S, D = x.shape
        H = 32
        Dh = D // H
        qkv = (lambda x, *d: x.transpose(*d))((x @ wqkv).reshape(B, S, 3, H, Dh), 2, 0, 3, 1, 4)
        q, k, v = qkv[0], qkv[1], qkv[2]
        scores = jnp.einsum("bhqd,bhkd->bhqk", q, k) * (Dh ** -0.5)
        p = _softmax(scores, axis=-1)
        o = jnp.einsum("bhqk,bhkd->bhqd", p, v)
        return (lambda x, *d: x.transpose(*d))(o, 0, 2, 1, 3).reshape(B, S, D) @ wo

    def _B_ref(x, w_gate, w_up, w_down):
        g = _silu(x @ w_gate)
        u = x @ w_up
        return (g * u) @ w_down

    x = A_x
    h = x + _A_ref(_layernorm(x, axis=-1), A_wqkv, A_wo)
    h2 = h + _B_ref(_layernorm(h, axis=-1), B_w_gate, B_w_up, B_w_down)
    return h2
```

```python
import math
import jax
import jax.numpy as jnp
from jax import lax
import jax.experimental.pallas as pl
import jax.experimental.pallas.tpu as pltpu

S, D, H, DH, F = 2048, 640, 32, 20, 1728
BQ = 1024
SUB = 512
CH = 128
RA = 512
RC = 512
FC = 512
EPS = 1e-5
QSCALE = (DH ** -0.5) * math.log2(math.e)
F32, BF16 = jnp.float32, jnp.bfloat16
NT = (((1,), (1,)), ((), ()))
TN = (((0,), (0,)), ((), ()))


def _ln(x, axis):
    mu = jnp.mean(x, axis=axis, keepdims=True)
    xc = x - mu
    var = jnp.mean(xc * xc, axis=axis, keepdims=True)
    return xc * lax.rsqrt(var + EPS)


def _kernel(x_hbm, wqkv_hbm, wo_hbm, wg_hbm, wu_hbm, wd_hbm, o_hbm,
            x_v, wqkv_v, wo_v, wg_v, wu_v, wd_v, wt_v, wot_v, wdt_v, xt_v, k9, q9, vt, qm, s_ref, at, ob, sems, osem):
    nA = S // RA
    cp_x = [pltpu.make_async_copy(x_hbm.at[pl.ds(i * RA, RA)], x_v.at[pl.ds(i * RA, RA)], sems.at[i]) for i in range(nA)]
    cp_qkv = pltpu.make_async_copy(wqkv_hbm, wqkv_v, sems.at[nA])
    cp_rest = [pltpu.make_async_copy(a, b, sems.at[nA + 1 + i]) for i, (a, b) in
               enumerate(((wo_hbm, wo_v), (wg_hbm, wg_v), (wu_hbm, wu_v), (wd_hbm, wd_v)))]
    cp_qkv.start()
    cp_x[0].start()
    cp_qkv.wait()
    for c in cp_x[1:]:
        c.start()
    wt_v[0:D, :] = (wqkv_v[:, 0:D].astype(F32).T).astype(BF16)
    wt_v[D:2 * D, :] = (wqkv_v[:, 2 * D:3 * D].astype(F32).T).astype(BF16)

    lane = lax.broadcasted_iota(jnp.int32, (RA, 128), 1)
    for i in range(nA):
        cp_x[i].wait()
        if i == nA - 1:
            for c in cp_rest:
                c.start()
        rows = pl.ds(i * RA, RA)
        xf = x_v[rows, :].astype(F32)
        xt_v[:, rows] = xf.T
        xn = _ln(xf, 1).astype(BF16)
        k = jnp.dot(xn, wqkv_v[:, D:2 * D], preferred_element_type=F32)
        kt = [k[:, j * 128:(j + 1) * 128] for j in range(5)]
        for j in range(5):
            k9[j, rows, :] = kt[j].astype(BF16)
        for j in range(4):
            k9[5 + j, rows, :] = jnp.where(lane >= 64, kt[j], kt[j + 1]).astype(BF16)
        q = lax.dot_general(wt_v[0:D, :], xn, NT, preferred_element_type=F32) * QSCALE
        q9[0:D, rows] = q.astype(BF16)
        v = lax.dot_general(wt_v[D:2 * D, :], xn, NT, preferred_element_type=F32)
        vt[:, rows] = v.astype(BF16).astype(F32)

    nq = S // BQ
    nu = nq * H
    nch = S // CH
    nsub = BQ // SUB
    row128 = lax.broadcasted_iota(jnp.int32, (128, BQ), 0)
    row24 = lax.broadcasted_iota(jnp.int32, (24, CH), 0)
    row24q = lax.broadcasted_iota(jnp.int32, (24, SUB), 0)

    def prep_q(u):
        h = u % H
        q0 = pl.multiple_of((u // H) * BQ, BQ)
        j = (h * DH) // 128
        off = (h * DH) % 128
        strad = off > 128 - DH
        hi = q9[pl.ds(pl.multiple_of(j * 128 + 64, 64), 64), pl.ds(q0, BQ)]
        lo = q9[pl.ds(pl.multiple_of((j + strad.astype(jnp.int32)) * 128, 64), 64), pl.ds(q0, BQ)]
        qt = jnp.concatenate([lo, hi], axis=0)
        keep = ((row128 - off) & 127) < DH
        qm[...] = jnp.where(keep, qt.astype(F32), 0.0).astype(BF16)
        return j + 5 * strad.astype(jnp.int32)

    def p1(t, c, b, m):
        cols = pl.ds(b * SUB, SUB)
        s = jnp.dot(k9[t, pl.ds(c * CH, CH), :], qm[:, cols], preferred_element_type=F32)
        s_ref[pl.ds(c * CH, CH), cols] = s
        return jnp.maximum(m, jnp.max(s.reshape(CH // 8, 8, SUB), axis=0))

    def p2(r0, one_row, c, b, m, acc):
        s = s_ref[pl.ds(c * CH, CH), pl.ds(b * SUB, SUB)]
        p = jnp.exp2(s - m).astype(BF16)
        v = jnp.where(row24 == one_row, 1.0, vt[pl.ds(r0, 24), pl.ds(c * CH, CH)])
        return acc + jnp.dot(v, p, preferred_element_type=F32)

    for c in cp_rest:
        c.wait()
    wot_v[...] = wo_v[...].astype(F32).T.astype(BF16)
    wdt_v[...] = wd_v[...].astype(F32).T.astype(BF16)
    ninf = jnp.full((8, SUB), -jnp.inf, F32)
    t = prep_q(0 * pl.program_id(0))
    ms = []
    for b in range(nsub):
        m = ninf
        for c in range(nch):
            m = p1(t, c, b, m)
        ms.append(jnp.max(m, axis=0, keepdims=True))

    def unit(u, ms):
        h = u % H
        q0 = (u // H) * BQ
        odd = (h % 2) == 1
        r0 = pl.multiple_of((h * DH) // 8 * 8, 8)
        one_row = jnp.where(odd, 0, 20)
        t = prep_q(jnp.minimum(u + 1, nu - 1))
        out = []
        for b in range(nsub):
            mn = ninf
            acc = jnp.zeros((24, SUB), F32)
            for c in range(nch):
                acc = p2(r0, one_row, c, b, ms[b], acc)
                mn = p1(t, c, b, mn)
            out.append(jnp.max(mn, axis=0, keepdims=True))
            l = jnp.where(odd, acc[0:1], acc[20:21])
            o = acc * (1.0 / l)
            cols = pl.ds(pl.multiple_of(q0 + b * SUB, SUB), SUB)
            old = at[pl.ds(r0, 8), cols]
            at[pl.ds(r0, 8), cols] = jnp.where(row24q[0:8] < jnp.where(odd, 4, 0), old, o[0:8])
            at[pl.ds(r0 + 8, 16), cols] = o[8:24]
        return tuple(out)

    lax.fori_loop(0, nu, unit, tuple(ms))

    def out_copy(i):
        return pltpu.make_async_copy(ob.at[i], o_hbm.at[pl.ds(i * RC, RC)], osem.at[i])

    def ffn(i, _):
        r = pl.multiple_of(i * RC, RC)
        a = at[:, pl.ds(r, RC)].astype(BF16)
        hh = xt_v[:, pl.ds(r, RC)] + jnp.dot(wot_v[...], a, preferred_element_type=F32)
        hn = _ln(hh, 0).astype(BF16)
        acc = hh
        for f0 in range(0, F, FC):
            fw = min(FC, F - f0)
            g = jnp.dot(wg_v[f0:f0 + fw, :], hn, preferred_element_type=F32)
            up = jnp.dot(wu_v[f0:f0 + fw, :], hn, preferred_element_type=F32)
            act = (g * jax.nn.sigmoid(g) * up).astype(BF16)
            acc = acc + jnp.dot(wdt_v[:, f0:f0 + fw], act, preferred_element_type=F32)
        ob[i] = acc.T.astype(BF16)
        out_copy(i).start()
        return 0
    lax.fori_loop(0, S // RC, ffn, 0)
    for i in range(S // RC):
        out_copy(i).wait()


@jax.jit
def pallas_sequential_preLN__mha_block__swiglu_ffn__prompt_kernel(A_x, A_wqkv, A_wo, B_x, B_w_gate, B_w_up, B_w_down):
    del B_x
    out = pl.pallas_call(
        _kernel,
        grid=(1,),
        in_specs=[pl.BlockSpec(memory_space=pltpu.HBM)] * 6,
        out_specs=pl.BlockSpec(memory_space=pltpu.HBM),
        out_shape=jax.ShapeDtypeStruct((S, D), BF16),
        scratch_shapes=[
            pltpu.VMEM((S, D), BF16), pltpu.VMEM((D, 3 * D), BF16), pltpu.VMEM((D, D), BF16),
            pltpu.VMEM((F, D), BF16), pltpu.VMEM((F, D), BF16), pltpu.VMEM((F, D), BF16),
            pltpu.VMEM((2 * D, D), BF16), pltpu.VMEM((D, D), BF16), pltpu.VMEM((D, F), BF16), pltpu.VMEM((D, S), F32),
            pltpu.VMEM((9, S, 128), BF16), pltpu.VMEM((D, S), BF16), pltpu.VMEM((D, S), F32),
            pltpu.VMEM((128, BQ), BF16), pltpu.VMEM((S, BQ), F32), pltpu.VMEM((D, S), F32),
            pltpu.VMEM((S // RC, RC, D), BF16),
            pltpu.SemaphoreType.DMA((S // RA + 5,)), pltpu.SemaphoreType.DMA((S // RC,)),
        ],
        compiler_params=pltpu.CompilerParams(vmem_limit_bytes=100 * 2 ** 20),
    )(A_x.reshape(S, D), A_wqkv, A_wo, B_w_gate.T, B_w_up.T, B_w_down)
    return out.reshape(1, S, D)
```

```python
import math
import jax
import jax.numpy as jnp
from jax import lax
import jax.experimental.pallas as pl
import jax.experimental.pallas.tpu as pltpu

S, D, H, DH, F = 2048, 640, 32, 20, 1728
BQ = 2048
SUB = 512
CH = 128
RA = 512
RC = 512
FC = 640
PS = -(-16 // (3 * -(-F // FC) - 1))
EPS = 1e-5
LOG2E = math.log2(math.e)
QSCALE = (DH ** -0.5) * math.log2(math.e)
F32, BF16 = jnp.float32, jnp.bfloat16
NT = (((1,), (1,)), ((), ()))


def _ln(x, axis):
    mu = jnp.mean(x, axis=axis, keepdims=True)
    xc = x - mu
    var = jnp.mean(xc * xc, axis=axis, keepdims=True)
    return xc * lax.rsqrt(var + EPS)


def _kernel(x_hbm, wqkv_hbm, wo_hbm, wg_hbm, wu_hbm, wd_hbm, o_hbm,
            x_v, wqkv_v, wo_v, wg_v, wu_v, wd_v, wt_v, wot_v, wdt_v, xt_v, xn_v, k9, q9, vt, qm, s_ref, at, ob, sems, osem):
    nA = S // RA
    cp_x = [pltpu.make_async_copy(x_hbm.at[pl.ds(i * RA, RA)], x_v.at[pl.ds(i * RA, RA)], sems.at[i]) for i in range(nA)]
    cp_w = [pltpu.make_async_copy(wqkv_hbm.at[:, pl.ds(i * D, D)], wqkv_v.at[:, pl.ds(i * D, D)], sems.at[nA + i])
            for i in range(3)]
    cp_rest = [pltpu.make_async_copy(a, b, sems.at[nA + 3 + i]) for i, (a, b) in
               enumerate(((wo_hbm, wo_v), (wg_hbm, wg_v), (wu_hbm, wu_v), (wd_hbm, wd_v)))]
    lane = lax.broadcasted_iota(jnp.int32, (RA, 128), 1)

    def norm(i):
        rows = pl.ds(i * RA, RA)
        xf = x_v[rows, :].astype(F32)
        xn_v[rows, :] = _ln(xf, 1).astype(BF16)

    def proj_k(i):
        rows = pl.ds(i * RA, RA)
        k = jnp.dot(xn_v[rows, :], wqkv_v[:, D:2 * D], preferred_element_type=F32)
        kt = [k[:, j * 128:(j + 1) * 128] for j in range(5)]
        for j in range(5):
            k9[j, pl.ds(i * RA // 2, RA // 2), :] = pltpu.bitcast(kt[j].astype(BF16), jnp.uint32)
        for j in range(4):
            k9[5 + j, pl.ds(i * RA // 2, RA // 2), :] = pltpu.bitcast(jnp.where(lane >= 64, kt[j], kt[j + 1]).astype(BF16), jnp.uint32)

    def proj_qv(i):
        rows = pl.ds(i * RA, RA)
        xn = xn_v[rows, :]
        q = lax.dot_general(wt_v[0:D, :], xn, NT, preferred_element_type=F32) * QSCALE
        q9[0:D, rows] = q.astype(BF16)
        v = lax.dot_general(wt_v[D:2 * D, :], xn, NT, preferred_element_type=F32)
        vt[:, rows] = v.astype(BF16).astype(F32)

    cp_x[0].start()
    cp_w[1].start()
    cp_x[0].wait()
    cp_x[1].start()
    norm(0)
    cp_w[1].wait()
    cp_w[0].start()
    cp_w[2].start()
    for c in cp_x[2:]:
        c.start()
    cp_x[1].wait()
    proj_k(0)
    norm(1)
    proj_k(1)
    cp_w[0].wait()
    cp_w[2].wait()
    for c in cp_x[2:]:
        c.wait()
    wt_v[0:D, :] = wqkv_v[:, 0:D].T
    wt_v[D:2 * D, :] = wqkv_v[:, 2 * D:3 * D].T
    for i in range(nA):
        if i + 2 < nA:
            norm(i + 2)
        proj_qv(i)
        if i + 2 < nA:
            proj_k(i + 2)

    nch = S // CH
    nsub = BQ // SUB
    row128 = lax.broadcasted_iota(jnp.int32, (128, BQ), 0)
    row24 = lax.broadcasted_iota(jnp.int32, (24, CH), 0)
    row24q = lax.broadcasted_iota(jnp.int32, (24, SUB), 0)

    def prep_q(u):
        h = u % H
        q0 = pl.multiple_of((u // H) * BQ, BQ)
        j = (h * DH) // 128
        off = (h * DH) % 128
        strad = off > 128 - DH
        hi = q9[pl.ds(pl.multiple_of(j * 128 + 64, 64), 64), pl.ds(q0, BQ)]
        lo = q9[pl.ds(pl.multiple_of((j + jnp.int32(strad)) * 128, 64), 64), pl.ds(q0, BQ)]
        qt = jnp.concatenate([lo, hi], axis=0)
        keep = ((row128 - off) & 127) < DH
        qm[...] = pltpu.bitcast(jnp.where(keep, qt.astype(F32), 0.0).astype(BF16), jnp.uint32)
        return j + 5 * jnp.int32(strad)

    def p1(t, c, b, m):
        cols = pl.ds(b * SUB, SUB)
        s = jnp.dot(pltpu.bitcast(k9[t, pl.ds(c * CH // 2, CH // 2), :], BF16), pltpu.bitcast(qm[:, cols], BF16), preferred_element_type=F32)
        s_ref[pl.ds(c * CH, CH), cols] = s
        return jnp.maximum(m, jnp.max(s.reshape(CH // 8, 8, SUB), axis=0))

    def p2(r0, one_row, c, b, m, acc):
        s = s_ref[pl.ds(c * CH, CH), pl.ds(b * SUB, SUB)]
        p = jnp.exp2(s - m).astype(BF16)
        v = jnp.where(row24 == one_row, 1.0, vt[pl.ds(r0, 24), pl.ds(c * CH, CH)])
        return acc + jnp.dot(v, p, preferred_element_type=F32)

    xt_v[...] = x_v[...].T
    ninf = jnp.full((8, SUB), -jnp.inf, F32)
    t = prep_q(0)
    ms = []
    for b in range(nsub):
        m = ninf
        for c in range(nch):
            m = p1(t, c, b, m)
        ms.append(jnp.max(m, axis=0, keepdims=True))

    def finish(h, b, acc):
        odd = (h % 2) == 1
        r0 = pl.multiple_of((h * DH) // 8 * 8, 8)
        l = jnp.where(odd, acc[0:1], acc[20:21])
        o = acc * (1.0 / l)
        cols = pl.ds(b * SUB, SUB)
        old = at[pl.ds(r0, 8), cols]
        at[pl.ds(r0, 8), cols] = jnp.where(row24q[0:8] < jnp.where(odd, 4, 0), old, o[0:8])
        at[pl.ds(r0 + 8, 16), cols] = o[8:24]

    def unit(h, ms):
        @pl.when(h == 1)
        def _():
            for c in cp_rest:
                c.start()

        r0 = pl.multiple_of((h * DH) // 8 * 8, 8)
        one_row = jnp.where((h % 2) == 1, 0, 20)
        t = prep_q(h + 1)
        out = []
        for b in range(nsub):
            mn = ninf
            acc = jnp.zeros((24, SUB), F32)
            for c in range(nch):
                acc = p2(r0, one_row, c, b, ms[b], acc)
                mn = p1(t, c, b, mn)
            out.append(jnp.max(mn, axis=0, keepdims=True))
            finish(h, b, acc)
        return tuple(out)

    ms = lax.fori_loop(0, H - 1, unit, tuple(ms))

    def out_copy(i):
        return pltpu.make_async_copy(ob.at[i], o_hbm.at[pl.ds(i * RC, RC)], osem.at[i])

    def last_head(b, cs, acc):
        for c in cs:
            acc = p2(((H - 1) * DH) // 8 * 8, 0, c, b, ms[b], acc)
        return acc

    def head_out(b, acc):
        finish(H - 1, b, acc)
        cols = pl.ds(b * RC, RC)
        hh = xt_v[:, cols].astype(F32) + jnp.dot(wot_v[...], at[:, cols].astype(BF16), preferred_element_type=F32)
        return hh, _ln(hh, 0).astype(BF16)

    for c in cp_rest:
        c.wait()
    wot_v[...] = wo_v[...].T
    wdt_v[...] = wd_v[...].T
    zero = jnp.zeros((24, SUB), F32)
    nxt = head_out(0, last_head(0, range(nch), zero))
    for b in range(nsub):
        acc, hn = nxt
        more = b + 1 < nsub
        pa = zero
        slot = 0
        def bg(pa, slot):
            if more:
                pa = last_head(b + 1, range(min(PS * slot, nch), min(PS * slot + PS, nch)), pa)
            return pa, slot + 1
        for f0 in range(0, F, FC):
            fw = min(FC, F - f0)
            g = jnp.dot(wg_v[f0:f0 + fw, :], hn, preferred_element_type=F32)
            pa, slot = bg(pa, slot)
            up = jnp.dot(wu_v[f0:f0 + fw, :], hn, preferred_element_type=F32)
            pa, slot = bg(pa, slot)
            act = (g * up / (1.0 + jnp.exp2(g * -LOG2E))).astype(BF16)
            if more and f0 + fw == F:
                nxt = head_out(b + 1, pa)
            acc = acc + jnp.dot(wdt_v[:, f0:f0 + fw], act, preferred_element_type=F32)
            pa, slot = bg(pa, slot)
        ob[b] = acc.astype(BF16).T
        out_copy(b).start()
    for i in range(S // RC):
        out_copy(i).wait()


@jax.jit
def pallas_sequential_preLN__mha_block__swiglu_ffn__prompt_kernel(A_x, A_wqkv, A_wo, B_x, B_w_gate, B_w_up, B_w_down):
    del B_x
    out = pl.pallas_call(
        _kernel,
        grid=(1,),
        in_specs=[pl.BlockSpec(memory_space=pltpu.HBM)] * 6,
        out_specs=pl.BlockSpec(memory_space=pltpu.HBM),
        out_shape=jax.ShapeDtypeStruct((S, D), BF16),
        scratch_shapes=[
            pltpu.VMEM((S, D), BF16), pltpu.VMEM((D, 3 * D), BF16), pltpu.VMEM((D, D), BF16),
            pltpu.VMEM((F, D), BF16), pltpu.VMEM((F, D), BF16), pltpu.VMEM((F, D), BF16),
            pltpu.VMEM((2 * D, D), BF16), pltpu.VMEM((D, D), BF16), pltpu.VMEM((D, F), BF16), pltpu.VMEM((D, S), BF16), pltpu.VMEM((S, D), BF16),
            pltpu.VMEM((9, S // 2, 128), jnp.uint32), pltpu.VMEM((D, S), BF16), pltpu.VMEM((D, S), F32),
            pltpu.VMEM((64, BQ), jnp.uint32), pltpu.VMEM((S, BQ), F32), pltpu.VMEM((D, S), F32),
            pltpu.VMEM((S // RC, RC, D), BF16),
            pltpu.SemaphoreType.DMA((S // RA + 7,)), pltpu.SemaphoreType.DMA((S // RC,)),
        ],
        compiler_params=pltpu.CompilerParams(vmem_limit_bytes=100 * 2 ** 20),
    )(A_x.reshape(S, D), A_wqkv, A_wo, B_w_gate.T, B_w_up.T, B_w_down)
    return out.reshape(1, S, D)
```
